```python
import jax
import jax.numpy as jnp

def _softmax(x, axis=-1):
    return jax.nn.softmax(x, axis=axis)

def _gelu(x):
    return jax.nn.gelu(x, approximate=True)

def _silu(x):
    return jax.nn.silu(x)

def _sigmoid(x):
    return jax.nn.sigmoid(x)

def _layernorm(x, axis=-1, eps=1e-05):
    m = jnp.mean(x, axis=axis, keepdims=True)
    v = jnp.var(x, axis=axis, keepdims=True)
    return (x - m) / jnp.sqrt(v + eps)

def _scatter_add(tgt, idx, src, axis=0):
    return tgt.at[idx].add(src)

def _segment_sum(src, seg, n):
    return jax.ops.segment_sum(src, seg, n)

class _Rng:

    def __init__(self, key):
        self._k = key

    def _next(self):
        self._k, sub = jax.random.split(self._k)
        return sub

    def normal(self, shape):
        return jax.random.normal(self._next(), shape, dtype=jnp.bfloat16)

    def randint(self, lo, hi, shape):
        return jax.random.randint(self._next(), shape, lo, hi, dtype=jnp.int32)

    def uniform(self, shape, lo=0.0, hi=1.0):
        return jax.random.uniform(self._next(), shape, jnp.bfloat16, lo, hi)

    def permutation(self, n):
        return jax.random.permutation(self._next(), n)
kernel_name = 'adaLN_cond__sliding_local_dilated__swiglu_ffn__prompt'

def setup_inputs():
    _rng = _Rng(jax.random.key(int.from_bytes(__import__("os").urandom(4), "little")))
    _w = lambda a: (lambda t: t.astype(jnp.bfloat16) if jnp.issubdtype(t.dtype, jnp.floating) else t)(jnp.asarray(a))

    def _A_setup():
        B, S, D = (1, 2048, 1024)
        return {'x': _w((lambda *s: _rng.normal(s) * 0.05)(B, S, D)), 'wqkv': _w((lambda *s: _rng.normal(s) * 0.05)(D, 3 * D)), 'wo': _w((lambda *s: _rng.normal(s) * 0.05)(D, D))}
    _A_in = _A_setup()

    def _B_setup():
        B, S, D, F = (1, 2048, 1024, 3584)
        return {'x': _w((lambda *s: _rng.normal(s) * 0.05)(B, S, D)), 'w_gate': _w((lambda *s: _rng.normal(s) * 0.05)(D, F)), 'w_up': _w((lambda *s: _rng.normal(s) * 0.05)(D, F)), 'w_down': _w((lambda *s: _rng.normal(s) * 0.05)(F, D))}
    _B_in = _B_setup()
    return {'A_x': _A_in['x'], 'A_wqkv': _A_in['wqkv'], 'A_wo': _A_in['wo'], 'B_x': _B_in['x'], 'B_w_gate': _B_in['w_gate'], 'B_w_up': _B_in['w_up'], 'B_w_down': _B_in['w_down'], 'c': _w((lambda *s: _rng.normal(s) * 0.05)(1, 1024)), 'w_mod': _w((lambda *s: _rng.normal(s) * 0.05)(1024, 6 * 1024) * 1024 ** (-0.5))}

def reference(A_x, A_wqkv, A_wo, B_x, B_w_gate, B_w_up, B_w_down, c, w_mod):

    def _A_ref(x, wqkv, wo):
        B, S, D = x.shape
        H = 32
        Dh = D // H
        W, dil = (8, 2)
        qkv = (lambda x, *d: x.transpose(*d))((x @ wqkv).reshape(B, S, 3, H, Dh), 2, 0, 3, 1, 4)
        q, k, v = (qkv[0], qkv[1], qkv[2])
        scale = Dh ** (-0.5)
        pos = jnp.arange(S)
        off = jnp.arange(W) * dil
        idx = pos[:, None] - off[None, :]
        mask = idx >= 0
        idx_c = jnp.where(mask, idx, 0).reshape(-1)
        kg = k[:, :, idx_c, :].reshape(B, H, S, W, Dh)
        vg = v[:, :, idx_c, :].reshape(B, H, S, W, Dh)
        logits = jnp.einsum('bhsd,bhswd->bhsw', q, kg) * scale
        logits = jnp.where(mask[None, None, :, :], logits, -1000000000.0)
        attn = _softmax(logits, axis=-1)
        o = jnp.einsum('bhsw,bhswd->bhsd', attn, vg)
        return (lambda x, *d: x.transpose(*d))(o, 0, 2, 1, 3).reshape(B, S, D) @ wo

    def _B_ref(x, w_gate, w_up, w_down):
        g = _silu(x @ w_gate)
        u = x @ w_up
        return g * u @ w_down
    x = A_x
    mod = (_silu(c) @ w_mod).reshape(c.shape[0], 6, 1, -1)
    sa, ca, ga, sb, cb, gb = (mod[:, 0].copy(), mod[:, 1].copy(), mod[:, 2].copy(), mod[:, 3].copy(), mod[:, 4].copy(), mod[:, 5].copy())
    h = _layernorm(x, axis=-1) * (1 + ca) + sa
    x = x + ga * _A_ref(h, A_wqkv, A_wo)
    h = _layernorm(x, axis=-1) * (1 + cb) + sb
    x = x + gb * _B_ref(h, B_w_gate, B_w_up, B_w_down)
    return x
```

```python
import functools

import jax
import jax.numpy as jnp
import jax.experimental.pallas as pl
import jax.experimental.pallas.tpu as pltpu

W_WIN, DIL = 8, 2
HALO = 16
LN_EPS = 1e-5


def _layernorm(x):
    m = jnp.mean(x, axis=-1, keepdims=True)
    d = x - m
    v = jnp.mean(d * d, axis=-1, keepdims=True)
    return d * jax.lax.rsqrt(v + LN_EPS)


def _dot(a, b):
    return jnp.dot(a, b, preferred_element_type=jnp.float32)


def _butterfly(t, axis, unit):
    n = t[0].shape[axis]
    idx = jax.lax.broadcasted_iota(jnp.int32, t[0].shape, axis)
    for b in range(3):
        sh = unit << b
        low = (idx & sh) == 0
        new = list(t)
        for g in range(8):
            if g & (1 << b):
                continue
            lo, hi = t[g], t[g | (1 << b)]
            new[g] = jnp.where(low, lo, pltpu.roll(hi, sh, axis))
            new[g | (1 << b)] = jnp.where(low, pltpu.roll(lo, n - sh, axis), hi)
        t = new
    return t


def _kernel(c_ref, x_ref, xn_ref, wmod_hbm, wqkv_hbm, wo_hbm, wg_hbm, wu_hbm, wd_hbm,
            o_ref,
            wmod_s, wqkv_s, wo_s, wg_s, wu_s, wd_s,
            mod_s, h_s, qkv_s, att_s, h2_s, acc_s, sems,
            *, TM, NT, R, NC, LR, PLACE, PR):
    i = pl.program_id(0)
    D = x_ref.shape[-1]
    NF, _, FC = wg_s.shape
    scale = (D // 32) ** -0.5
    f32, bf16 = jnp.float32, jnp.bfloat16
    nch = TM // R
    per = -(-nch // NF)

    def c_mod(n):
        return pltpu.make_async_copy(
            wmod_hbm.at[:, pl.ds(pl.multiple_of(n * D, D), D)], wmod_s.at[n], sems.at[n])

    def c_qkv(n):
        return pltpu.make_async_copy(
            wqkv_hbm.at[:, pl.ds(pl.multiple_of(n * D, D), D)], wqkv_s.at[n], sems.at[6 + n])

    def c_wo():
        return pltpu.make_async_copy(wo_hbm, wo_s, sems.at[9])

    def c_ffn(f):
        f0 = pl.multiple_of(f * FC, FC)
        return (pltpu.make_async_copy(wg_hbm.at[:, pl.ds(f0, FC)], wg_s.at[f], sems.at[10 + 3 * f]),
                pltpu.make_async_copy(wu_hbm.at[:, pl.ds(f0, FC)], wu_s.at[f], sems.at[11 + 3 * f]),
                pltpu.make_async_copy(wd_hbm.at[pl.ds(f0, FC), :], wd_s.at[f], sems.at[12 + 3 * f]))

    def start(*cs):
        for c in cs:
            c.start()

    def mod_part(n):
        cv = c_ref[...].astype(f32)
        sc = jnp.broadcast_to((cv * jax.nn.sigmoid(cv)).astype(bf16), (16, D))
        mod_s[n] = _dot(sc, wmod_s[n])[0:8]

    def mod(n):
        return mod_s[n, 0:1, :]

    def permute_cols(n):
        def body(r, _):
            rows = pl.ds(pl.multiple_of(r * PR, PR), PR)
            t = [pltpu.bitcast(wqkv_s[n, rows, g * 128:(g + 1) * 128], jnp.uint32) for g in range(8)]
            t = _butterfly(t, 1, 4)
            for g in range(8):
                wqkv_s[n, rows, g * 128:(g + 1) * 128] = pltpu.bitcast(t[g], bf16)
        jax.lax.fori_loop(0, D // PR, body, None)

    def permute_wo():
        def body(n, _):
            cs = pl.ds(pl.multiple_of(n * 128, 128), 128)
            t = [pltpu.bitcast(wo_s[g * 128:(g + 1) * 128, cs], jnp.uint32) for g in range(8)]
            t = _butterfly(t, 0, 2)
            for g in range(8):
                wo_s[g * 128:(g + 1) * 128, cs] = pltpu.bitcast(t[g], bf16)
        jax.lax.fori_loop(0, D // 128, body, None)

    def ln1(src):
        sa, ca1 = mod(0), 1.0 + mod(1)
        for r0 in range(0, TM, LR):
            xv = src[r0:r0 + LR, :].astype(f32)
            h_s[r0:r0 + LR, :] = (_layernorm(xv) * ca1 + sa).astype(bf16)

    def qkv(n):
        qkv_s[n, :, 0:HALO, :] = qkv_s[n, :, TM:TM + HALO, :]
        for c0 in range(0, D, NC):
            y = _dot(h_s[...], wqkv_s[n, :, c0:c0 + NC])
            for jj in range(NC // 128):
                qkv_s[n, c0 // 128 + jj, HALO:HALO + TM, :] = y[:, jj * 128:(jj + 1) * 128]

    def attn(ch):
        r0 = pl.multiple_of(ch * R, R)

        def rows(n, j, back):
            return qkv_s[n, j, pl.ds(r0 + (HALO - back), R), :]
        l = [None] * W_WIN
        for j in range(8):
            qj = rows(0, j, 0)
            for w in range(W_WIN):
                p = qj * rows(1, j, DIL * w)
                l[w] = p if l[w] is None else l[w] + p
        lane = jax.lax.broadcasted_iota(jnp.int32, (R, 128), 1)
        pos = jax.lax.broadcasted_iota(jnp.int32, (R, 128), 0) + (i * TM + r0)
        b0, b1 = (lane & 1) == 0, (lane & 2) == 0
        for w in range(W_WIN):
            t = l[w]
            t = t + jnp.where(b0, pltpu.roll(t, 127, 1), pltpu.roll(t, 1, 1))
            t = t + jnp.where(b1, pltpu.roll(t, 126, 1), pltpu.roll(t, 2, 1))
            t = t * scale
            l[w] = jnp.where(pos >= DIL * w, t, -1e9) if w else t
        m = functools.reduce(jnp.maximum, l)
        e = [jnp.exp(t - m) for t in l]
        inv = 1.0 / functools.reduce(jnp.add, e)
        e = [t * inv for t in e]
        for j in range(8):
            acc = None
            for w in range(W_WIN):
                p = e[w] * rows(2, j, DIL * w)
                acc = p if acc is None else acc + p
            att_s[pl.ds(r0, R), j * 128:(j + 1) * 128] = acc.astype(bf16)

    def out_proj():
        ga = mod(2)
        for c0 in range(0, D, NC):
            cs = slice(c0, c0 + NC)
            acc_s[:, cs] = x_ref[:, cs].astype(f32) + ga[:, cs] * _dot(att_s[...], wo_s[:, cs])

    def ln2(base, nrows):
        sb, cb1 = mod(3), 1.0 + mod(4)
        for r0 in range(0, nrows, LR):
            rows = pl.ds(base + r0, LR)
            h2_s[rows, :] = (_layernorm(acc_s[rows, :]) * cb1 + sb).astype(bf16)

    def ffn(f, side):
        a = []
        slot = iter(PLACE)
        t_side = iter(range(per))

        def do_side():
            for _ in range(next(slot)):
                side(next(t_side))
        for c0 in range(0, FC, NC):
            do_side()
            g = _dot(h2_s[...], wg_s[f, :, c0:c0 + NC])
            u = _dot(h2_s[...], wu_s[f, :, c0:c0 + NC])
            t = 0.5 * g
            a.append(((t * jnp.tanh(t) + t) * u).astype(bf16))
        a = jnp.concatenate(a, axis=1)
        gb = mod(5)
        for c0 in range(0, D, NC):
            do_side()
            cs = slice(c0, c0 + NC)
            res = acc_s[:, cs] + gb[:, cs] * _dot(a, wd_s[f, :, cs])
            acc_s[:, cs] = res
            o_ref[:, cs] = res.astype(o_ref.dtype)
        for t in t_side:
            side(t)

    first = i == 0

    @pl.when(first)
    def _():
        start(c_mod(0), c_mod(1))
        qkv_s[:, :, TM:TM + HALO, :] = jnp.zeros((3, 8, HALO, 128), f32)
        acc_s[...] = jnp.zeros_like(acc_s)
        mod_s[3:5] = jnp.zeros((2, 8, D), f32)

        def body(n, _):
            c_mod(n).wait()
            start(c_qkv(n))
            mod_part(n)
        jax.lax.fori_loop(0, 2, body, None)
        ln1(x_ref)

    @pl.when(i < NT)
    def _():
        third = -(-TM // (3 * LR)) * LR

        def body(n, _):
            @pl.when(first)
            def _():
                c_qkv(n).wait()
                pl.when(n == 0)(lambda: start(c_qkv(2)))
                pl.when(n == 1)(lambda: start(c_wo(), c_mod(2)))
                pl.when(n == 2)(lambda: start(c_mod(3), c_mod(4)))
                permute_cols(n)
            ln2(pl.multiple_of(jnp.minimum(n * third, TM - third), LR), third)
            qkv(n)
        jax.lax.fori_loop(0, 3, body, None)

    pl.when(i == NT)(lambda: ln2(0, TM))

    @pl.when(first)
    def _():
        c_wo().wait()
        start(c_mod(5), *c_ffn(0))
        permute_wo()

        def body(n, _):
            c_mod(n).wait()
            pl.when(n < 5)(lambda: start(*c_ffn(n - 1)))
            mod_part(n)
            for t in range(nch // 4):
                attn((n - 2) * (nch // 4) + t)
        jax.lax.fori_loop(2, 6, body, None)

    @pl.when(i > 0)
    def _():
        def body(f, _):
            @pl.when(i == 1)
            def _():
                for c in c_ffn(f):
                    c.wait()
                pl.when(f + 4 < NF)(lambda: start(*c_ffn(f + 4)))
            ffn(f, lambda t: attn(jnp.minimum(f * per + t, nch - 1)))
        jax.lax.fori_loop(0, NF, body, None)

    @pl.when(i < NT)
    def _():
        ln1(xn_ref)
        out_proj()


def _build(S, D, F, TM=256, FC=512, R=16, NC=256, LR=32, PLACE=(0,) * 12, PR=64):
    NT = S // TM
    NF = F // FC
    assert S % TM == 0 and NT >= 2 and F % FC == 0 and NF >= 4 and D == 1024 and TM % R == 0
    bf, f32 = jnp.bfloat16, jnp.float32
    any_spec = pl.BlockSpec(memory_space=pl.ANY)
    call = pl.pallas_call(
        functools.partial(_kernel, TM=TM, NT=NT, R=R, NC=NC, LR=LR, PLACE=PLACE, PR=PR),
        grid=(NT + 1,),
        in_specs=[pl.BlockSpec((1, D), lambda i: (0, 0)),
                  pl.BlockSpec((TM, D), lambda i: (jnp.minimum(i, NT - 1), 0)),
                  pl.BlockSpec((TM, D), lambda i: (jnp.minimum(i + 1, NT - 1), 0))] + [any_spec] * 6,
        out_specs=pl.BlockSpec((TM, D), lambda i: (jnp.maximum(i - 1, 0), 0)),
        out_shape=jax.ShapeDtypeStruct((S, D), bf),
        scratch_shapes=[
            pltpu.VMEM((6, D, D), bf), pltpu.VMEM((3, D, D), bf), pltpu.VMEM((D, D), bf),
            pltpu.VMEM((NF, D, FC), bf), pltpu.VMEM((NF, D, FC), bf), pltpu.VMEM((NF, FC, D), bf),
            pltpu.VMEM((6, 8, D), f32), pltpu.VMEM((TM, D), bf),
            pltpu.VMEM((3, 8, TM + HALO, 128), f32), pltpu.VMEM((TM, D), bf),
            pltpu.VMEM((TM, D), bf), pltpu.VMEM((TM, D), f32),
            pltpu.SemaphoreType.DMA((10 + 3 * NF,)),
        ],
        compiler_params=pltpu.CompilerParams(
            dimension_semantics=("arbitrary",), vmem_limit_bytes=100 * 1024 * 1024),
    )
    return lambda c, x, *w: call(c, x, x, *w)


@jax.jit
def pallas_adaLN_cond__sliding_local_dilated__swiglu_ffn__prompt_kernel(
    A_x: jax.Array,
    A_wqkv: jax.Array,
    A_wo: jax.Array,
    B_x: jax.Array,
    B_w_gate: jax.Array,
    B_w_up: jax.Array,
    B_w_down: jax.Array,
    c: jax.Array,
    w_mod: jax.Array,
):
    del B_x
    B, S, D = A_x.shape
    assert B == 1
    out = _build(S, D, B_w_gate.shape[1])(
        c, A_x.reshape(S, D), w_mod, A_wqkv, A_wo, B_w_gate, B_w_up, B_w_down)
    return out.reshape(B, S, D)
```

```python
import functools

import jax
import jax.numpy as jnp
import jax.experimental.pallas as pl
import jax.experimental.pallas.tpu as pltpu

W_WIN, DIL = 8, 2
HALO = 16
LN_EPS = 1e-5


def _layernorm(x):
    m = jnp.mean(x, axis=-1, keepdims=True)
    d = x - m
    v = jnp.mean(d * d, axis=-1, keepdims=True)
    return d * jax.lax.rsqrt(v + LN_EPS)


def _dot(a, b):
    return jnp.dot(a, b, preferred_element_type=jnp.float32)


def _block_transpose(t, axis, unit):
    n = t[0].shape[axis]
    idx = jax.lax.broadcasted_iota(jnp.int32, t[0].shape, axis)
    t = [pltpu.roll(x, unit * g, axis) if g else x for g, x in enumerate(t)]
    for b in range(3):
        bit = (idx & (unit << b)) != 0
        t = [jnp.where(bit, t[(g + (1 << b)) % 8], t[g]) for g in range(8)]
    return [pltpu.roll(t[-s % 8], n - unit * s, axis) if s else t[0] for s in range(8)]


def _kernel(c_ref, x_ref, xn_ref, wmod_hbm, wqkv_hbm, wo_hbm, wg_hbm, wu_hbm, wd_hbm,
            o_ref,
            wmod_s, wqkv_s, wo_s, wg_s, wu_s, wd_s,
            mod_s, h_s, qkv_s, att_s, h2_s, acc_s, sems,
            *, TM, NT, R, NC, LR, PR, AU, QU, R0):
    i = pl.program_id(0)
    D = x_ref.shape[-1]
    NF, _, FC = wg_s.shape
    scale = (D // 32) ** -0.5
    f32, bf16 = jnp.float32, jnp.bfloat16
    nch = TM // R
    per = -(-nch // NF)

    def c_mod(n):
        return pltpu.make_async_copy(
            wmod_hbm.at[:, pl.ds(pl.multiple_of(n * D, D), D)], wmod_s.at[n], sems.at[n])

    def c_qkv(n):
        return pltpu.make_async_copy(
            wqkv_hbm.at[:, pl.ds(pl.multiple_of(n * D, D), D)], wqkv_s.at[n], sems.at[6 + n])

    def c_wo():
        return pltpu.make_async_copy(wo_hbm, wo_s, sems.at[9])

    def c_ffn(f):
        f0 = pl.multiple_of(f * FC, FC)
        return (pltpu.make_async_copy(wg_hbm.at[:, pl.ds(f0, FC)], wg_s.at[f], sems.at[10 + 3 * f]),
                pltpu.make_async_copy(wu_hbm.at[:, pl.ds(f0, FC)], wu_s.at[f], sems.at[11 + 3 * f]),
                pltpu.make_async_copy(wd_hbm.at[pl.ds(f0, FC), :], wd_s.at[f], sems.at[12 + 3 * f]))

    def start(*cs):
        for c in cs:
            c.start()

    def mod_part(n):
        cv = c_ref[...].astype(f32)
        sc = jnp.broadcast_to((cv * jax.nn.sigmoid(cv)).astype(bf16), (16, D))
        mod_s[n] = _dot(sc, wmod_s[n])[0:8]

    def mod(n):
        return mod_s[n, 0:1, :]

    def permute_cols(n):
        def body(r, _):
            rows = pl.ds(pl.multiple_of(r * PR, PR), PR)
            t = [pltpu.bitcast(wqkv_s[n, rows, g * 128:(g + 1) * 128], jnp.uint32) for g in range(8)]
            t = _block_transpose(t, 1, 4)
            for g in range(8):
                wqkv_s[n, rows, g * 128:(g + 1) * 128] = pltpu.bitcast(t[g], bf16)
        jax.lax.fori_loop(0, D // PR, body, None)

    def permute_wo():
        def body(n, _):
            cs = pl.ds(pl.multiple_of(n * 128, 128), 128)
            t = [pltpu.bitcast(wo_s[g * 128:(g + 1) * 128, cs], jnp.uint32) for g in range(8)]
            t = _block_transpose(t, 0, 2)
            for g in range(8):
                wo_s[g * 128:(g + 1) * 128, cs] = pltpu.bitcast(t[g], bf16)
        jax.lax.fori_loop(0, D // 128, body, None)

    def ln1(src, base, nrows):
        sa, ca1 = mod(0), 1.0 + mod(1)
        for r0 in range(0, nrows, LR):
            rows = pl.ds(base + r0, min(LR, nrows - r0))
            h_s[rows, :] = (_layernorm(src[rows, :].astype(f32)) * ca1 + sa).astype(bf16)

    def qkv(n):
        qkv_s[n, :, 0:HALO, :] = qkv_s[n, :, TM:TM + HALO, :]
        for c0 in range(0, D, NC):
            y = _dot(h_s[...], wqkv_s[n, :, c0:c0 + NC])
            for jj in range(NC // 128):
                qkv_s[n, c0 // 128 + jj, HALO:HALO + TM, :] = y[:, jj * 128:(jj + 1) * 128]

    def attn(ch, R=R):
        r0 = pl.multiple_of(ch * R, R)

        def rows(n, j, back):
            return qkv_s[n, j, pl.ds(r0 + (HALO - back), R), :]
        l = [None] * W_WIN
        for j in range(8):
            qj = rows(0, j, 0)
            for w in range(W_WIN):
                p = qj * rows(1, j, DIL * w)
                l[w] = p if l[w] is None else l[w] + p
        lane = jax.lax.broadcasted_iota(jnp.int32, (R, 128), 1)
        pos = jax.lax.broadcasted_iota(jnp.int32, (R, 128), 0) + (i * TM + r0)
        b0, b1 = (lane & 1) == 0, (lane & 2) == 0
        for w in range(W_WIN):
            t = l[w]
            t = t + jnp.where(b0, pltpu.roll(t, 127, 1), pltpu.roll(t, 1, 1))
            t = t + jnp.where(b1, pltpu.roll(t, 126, 1), pltpu.roll(t, 2, 1))
            t = t * scale
            l[w] = jnp.where(pos >= DIL * w, t, -1e9) if w else t
        m = functools.reduce(jnp.maximum, l)
        e = [jnp.exp(t - m) for t in l]
        inv = 1.0 / functools.reduce(jnp.add, e)
        e = [t * inv for t in e]
        for j in range(8):
            acc = None
            for w in range(W_WIN):
                p = e[w] * rows(2, j, DIL * w)
                acc = p if acc is None else acc + p
            att_s[pl.ds(r0, R), j * 128:(j + 1) * 128] = acc.astype(bf16)

    def out_proj():
        ga = mod(2)
        for c0 in range(0, D, NC):
            cs = slice(c0, c0 + NC)
            acc_s[:, cs] = x_ref[:, cs].astype(f32) + ga[:, cs] * _dot(att_s[...], wo_s[:, cs])

    def ln2(base, nrows):
        sb, cb1 = mod(3), 1.0 + mod(4)
        for r0 in range(0, nrows, LR):
            rows = pl.ds(base + r0, min(LR, nrows - r0))
            h2_s[rows, :] = (_layernorm(acc_s[rows, :]) * cb1 + sb).astype(bf16)

    def ffn(f):
        a = []
        for c0 in range(0, FC, NC):
            cs = slice(c0, min(c0 + NC, FC))
            g = _dot(h2_s[...], wg_s[f, :, cs])
            u = _dot(h2_s[...], wu_s[f, :, cs])
            t = 0.5 * g
            a.append(((t * jnp.tanh(t) + t) * u).astype(bf16))
        a = jnp.concatenate(a, axis=1)
        gb = mod(5)
        for c0 in range(0, D, NC):
            cs = slice(c0, c0 + NC)
            res = acc_s[:, cs] + gb[:, cs] * _dot(a, wd_s[f, :, cs])
            acc_s[:, cs] = res
            o_ref[:, cs] = res.astype(o_ref.dtype)

    def share(k, parts):
        size = -(-TM // (parts * 16)) * 16
        return pl.multiple_of(jnp.minimum(k * size, TM - size), 16), size

    first = i == 0

    @pl.when(first)
    def _():
        start(c_qkv(0), c_qkv(1))
        qkv_s[:, :, TM:TM + HALO, :] = jnp.zeros((3, 8, HALO, 128), f32)
        acc_s[...] = jnp.zeros_like(acc_s)
        mod_s[3:5] = jnp.zeros((2, 8, D), f32)

        def perm_body(n, _):
            c_qkv(n).wait()
            pl.when(n == 0)(lambda: start(c_qkv(2), c_mod(0)))
            pl.when(n == 1)(lambda: start(c_mod(1)))
            pl.when(n == 2)(lambda: start(c_wo()))
            permute_cols(n)
        jax.lax.fori_loop(0, 3, perm_body, None)

        def mod_body(n, _):
            c_mod(n).wait()
            start(c_mod(2 + n))
            mod_part(n)
        jax.lax.fori_loop(0, 2, mod_body, None)
        start(c_mod(4))
        ln1(x_ref, 0, TM)

    @pl.when(i < NT)
    def _():
        if QU:
            ln2(0, TM)
            for n in range(3):
                qkv(n)
        else:
            def body(n, _):
                ln2(*share(n, 3))
                qkv(n)
            jax.lax.fori_loop(0, 3, body, None)

    pl.when(i == NT)(lambda: ln2(0, TM))

    @pl.when(first)
    def _():
        c_wo().wait()
        start(c_mod(5), *c_ffn(0))
        permute_wo()
        def attn_body(t, _):
            for u in range(AU):
                attn(t * AU + u, R0)
            ln1(xn_ref, *share(t, TM // (R0 * AU)))
        jax.lax.fori_loop(0, TM // (R0 * AU), attn_body, None)

        def body(n, _):
            c_mod(n).wait()
            mod_part(n)
        jax.lax.fori_loop(2, 5, body, None)

    @pl.when(i == 1)
    def _():
        c_mod(5).wait()
        start(*c_ffn(1))
        mod_part(5)

    @pl.when(i > 0)
    def _():
        def body(f, _):
            @pl.when(i == 1)
            def _():
                for c in c_ffn(f):
                    c.wait()
                pl.when(f + 2 < NF)(lambda: start(*c_ffn(f + 2)))
            ffn(f)
            for t in range(per):
                attn(jnp.minimum(f * per + t, nch - 1))
            ln1(xn_ref, *share(f, NF))
        jax.lax.fori_loop(0, NF, body, None)

    @pl.when(i < NT)
    def _():
        out_proj()


def _build(S, D, F, TM=256, FC=1792, R=8, NC=256, LR=32, PR=256, AU=2, QU=True, R0=8):
    NT = S // TM
    NF = F // FC
    assert S % TM == 0 and NT >= 2 and F % FC == 0 and NF >= 2 and D == 1024 and TM % R == 0
    bf, f32 = jnp.bfloat16, jnp.float32
    any_spec = pl.BlockSpec(memory_space=pl.ANY)
    call = pl.pallas_call(
        functools.partial(_kernel, TM=TM, NT=NT, R=R, NC=NC, LR=LR, PR=PR, AU=AU, QU=QU, R0=R0),
        grid=(NT + 1,),
        in_specs=[pl.BlockSpec((1, D), lambda i: (0, 0)),
                  pl.BlockSpec((TM, D), lambda i: (jnp.minimum(i, NT - 1), 0)),
                  pl.BlockSpec((TM, D), lambda i: (jnp.minimum(i + 1, NT - 1), 0))] + [any_spec] * 6,
        out_specs=pl.BlockSpec((TM, D), lambda i: (jnp.maximum(i - 1, 0), 0)),
        out_shape=jax.ShapeDtypeStruct((S, D), bf),
        scratch_shapes=[
            pltpu.VMEM((6, D, D), bf), pltpu.VMEM((3, D, D), bf), pltpu.VMEM((D, D), bf),
            pltpu.VMEM((NF, D, FC), bf), pltpu.VMEM((NF, D, FC), bf), pltpu.VMEM((NF, FC, D), bf),
            pltpu.VMEM((6, 8, D), f32), pltpu.VMEM((TM, D), bf),
            pltpu.VMEM((3, 8, TM + HALO, 128), f32), pltpu.VMEM((TM, D), bf),
            pltpu.VMEM((TM, D), bf), pltpu.VMEM((TM, D), f32),
            pltpu.SemaphoreType.DMA((10 + 3 * NF,)),
        ],
        compiler_params=pltpu.CompilerParams(
            dimension_semantics=("arbitrary",), vmem_limit_bytes=100 * 1024 * 1024),
    )
    return lambda c, x, *w: call(c, x, x, *w)


@jax.jit
def pallas_adaLN_cond__sliding_local_dilated__swiglu_ffn__prompt_kernel(
    A_x: jax.Array,
    A_wqkv: jax.Array,
    A_wo: jax.Array,
    B_x: jax.Array,
    B_w_gate: jax.Array,
    B_w_up: jax.Array,
    B_w_down: jax.Array,
    c: jax.Array,
    w_mod: jax.Array,
):
    del B_x
    B, S, D = A_x.shape
    assert B == 1
    out = _build(S, D, B_w_gate.shape[1])(
        c, A_x.reshape(S, D), w_mod, A_wqkv, A_wo, B_w_gate, B_w_up, B_w_down)
    return out.reshape(B, S, D)
```

```python
import functools

import jax
import jax.numpy as jnp
import jax.experimental.pallas as pl
import jax.experimental.pallas.tpu as pltpu

W_WIN, DIL = 8, 2
HALO = 16
LN_EPS = 1e-5


def _layernorm(x):
    m = jnp.mean(x, axis=-1, keepdims=True)
    d = x - m
    v = jnp.mean(d * d, axis=-1, keepdims=True)
    return d * jax.lax.rsqrt(v + LN_EPS)


def _dot(a, b):
    return jnp.dot(a, b, preferred_element_type=jnp.float32)


def _block_transpose(t, axis, unit):
    n = t[0].shape[axis]
    idx = jax.lax.broadcasted_iota(jnp.int32, t[0].shape, axis)
    t = [pltpu.roll(x, unit * g, axis) if g else x for g, x in enumerate(t)]
    for b in range(3):
        bit = (idx & (unit << b)) != 0
        t = [jnp.where(bit, t[(g + (1 << b)) % 8], t[g]) for g in range(8)]
    return [pltpu.roll(t[-s % 8], n - unit * s, axis) if s else t[0] for s in range(8)]


def _kernel(c_hbm, x_hbm, wmod_hbm, wqkv_hbm, wo_hbm, wg_hbm, wu_hbm, wd_hbm,
            o_ref,
            wmod_s, wqkv_s, wo_s, wg_s, wu_s, wd_s,
            mod_s, h_s, qkv_s, att_s, h2_s, acc_s, c_ref, x_s, sems, io_sems,
            *, TM, NT, R, NC, LR, PR, AU, QU, R0):
    i = pl.program_id(0)
    D = x_s.shape[-1]
    NF, _, FC = wg_s.shape
    scale = (D // 32) ** -0.5
    f32, bf16 = jnp.float32, jnp.bfloat16
    nch = TM // R
    per = -(-nch // NF)

    def c_mod(n):
        return pltpu.make_async_copy(
            wmod_hbm.at[:, pl.ds(pl.multiple_of(n * D, D), D)], wmod_s.at[n], sems.at[n])

    def c_qkv(n):
        return pltpu.make_async_copy(
            wqkv_hbm.at[:, pl.ds(pl.multiple_of(n * D, D), D)], wqkv_s.at[n], sems.at[6 + n])

    def c_wo():
        return pltpu.make_async_copy(wo_hbm, wo_s, sems.at[9])

    def c_ffn(f):
        f0 = pl.multiple_of(f * FC, FC)
        return (pltpu.make_async_copy(wg_hbm.at[:, pl.ds(f0, FC)], wg_s.at[f], sems.at[10 + 3 * f]),
                pltpu.make_async_copy(wu_hbm.at[:, pl.ds(f0, FC)], wu_s.at[f], sems.at[11 + 3 * f]),
                pltpu.make_async_copy(wd_hbm.at[pl.ds(f0, FC), :], wd_s.at[f], sems.at[12 + 3 * f]))

    def c_x(t):
        return pltpu.make_async_copy(
            x_hbm.at[pl.ds(pl.multiple_of(t * TM, TM), TM)], x_s.at[t], io_sems.at[t])

    def c_c():
        return pltpu.make_async_copy(c_hbm, c_ref, io_sems.at[NT])

    def start(*cs):
        for c in cs:
            c.start()

    def mod_part(n):
        cv = c_ref[...].astype(f32)
        sc = jnp.broadcast_to((cv * jax.nn.sigmoid(cv)).astype(bf16), (16, D))
        mod_s[n] = _dot(sc, wmod_s[n])[0:8]

    def mod(n):
        return mod_s[n, 0:1, :]

    def permute_cols(n):
        def body(r, _):
            rows = pl.ds(pl.multiple_of(r * PR, PR), PR)
            t = [pltpu.bitcast(wqkv_s[n, rows, g * 128:(g + 1) * 128], jnp.uint32) for g in range(8)]
            t = _block_transpose(t, 1, 4)
            for g in range(8):
                wqkv_s[n, rows, g * 128:(g + 1) * 128] = pltpu.bitcast(t[g], bf16)
        jax.lax.fori_loop(0, D // PR, body, None)

    def permute_wo():
        def body(n, _):
            cs = pl.ds(pl.multiple_of(n * 128, 128), 128)
            t = [pltpu.bitcast(wo_s[g * 128:(g + 1) * 128, cs], jnp.uint32) for g in range(8)]
            t = _block_transpose(t, 0, 2)
            for g in range(8):
                wo_s[g * 128:(g + 1) * 128, cs] = pltpu.bitcast(t[g], bf16)
        jax.lax.fori_loop(0, D // 128, body, None)

    def ln1(tile, base, nrows):
        sa, ca1 = mod(0), 1.0 + mod(1)
        for r0 in range(0, nrows, LR):
            rows = pl.ds(base + r0, min(LR, nrows - r0))
            h_s[rows, :] = (_layernorm(x_s[tile, rows, :].astype(f32)) * ca1 + sa).astype(bf16)

    def qkv(n):
        qkv_s[n, :, 0:HALO, :] = qkv_s[n, :, TM:TM + HALO, :]
        for c0 in range(0, D, NC):
            y = _dot(h_s[...], wqkv_s[n, :, c0:c0 + NC])
            for jj in range(NC // 128):
                qkv_s[n, c0 // 128 + jj, HALO:HALO + TM, :] = y[:, jj * 128:(jj + 1) * 128]

    def attn(ch, R=R):
        r0 = pl.multiple_of(ch * R, R)

        def rows(n, j, back):
            return qkv_s[n, j, pl.ds(r0 + (HALO - back), R), :]
        l = [None] * W_WIN
        for j in range(8):
            qj = rows(0, j, 0)
            for w in range(W_WIN):
                p = qj * rows(1, j, DIL * w)
                l[w] = p if l[w] is None else l[w] + p
        lane = jax.lax.broadcasted_iota(jnp.int32, (R, 128), 1)
        pos = jax.lax.broadcasted_iota(jnp.int32, (R, 128), 0) + (i * TM + r0)
        b0, b1 = (lane & 1) == 0, (lane & 2) == 0
        for w in range(W_WIN):
            t = l[w]
            t = t + jnp.where(b0, pltpu.roll(t, 127, 1), pltpu.roll(t, 1, 1))
            t = t + jnp.where(b1, pltpu.roll(t, 126, 1), pltpu.roll(t, 2, 1))
            t = t * scale
            l[w] = jnp.where(pos >= DIL * w, t, -1e9) if w else t
        m = functools.reduce(jnp.maximum, l)
        e = [jnp.exp(t - m) for t in l]
        inv = 1.0 / functools.reduce(jnp.add, e)
        e = [t * inv for t in e]
        for j in range(8):
            acc = None
            for w in range(W_WIN):
                p = e[w] * rows(2, j, DIL * w)
                acc = p if acc is None else acc + p
            att_s[pl.ds(r0, R), j * 128:(j + 1) * 128] = acc.astype(bf16)

    def out_proj():
        ga = mod(2)
        for c0 in range(0, D, NC):
            cs = slice(c0, c0 + NC)
            acc_s[:, cs] = x_s[i, :, cs].astype(f32) + ga[:, cs] * _dot(att_s[...], wo_s[:, cs])

    def ln2(base, nrows):
        sb, cb1 = mod(3), 1.0 + mod(4)
        for r0 in range(0, nrows, LR):
            rows = pl.ds(base + r0, min(LR, nrows - r0))
            h2_s[rows, :] = (_layernorm(acc_s[rows, :]) * cb1 + sb).astype(bf16)

    def ffn(f):
        a = []
        for c0 in range(0, FC, NC):
            cs = slice(c0, min(c0 + NC, FC))
            g = _dot(h2_s[...], wg_s[f, :, cs])
            u = _dot(h2_s[...], wu_s[f, :, cs])
            t = 0.5 * g
            a.append(((t * jnp.tanh(t) + t) * u).astype(bf16))
        a = jnp.concatenate(a, axis=1)
        gb = mod(5)
        for c0 in range(0, D, NC):
            cs = slice(c0, c0 + NC)
            res = acc_s[:, cs] + gb[:, cs] * _dot(a, wd_s[f, :, cs])
            acc_s[:, cs] = res
            o_ref[:, cs] = res.astype(o_ref.dtype)

    def share(k, parts):
        size = -(-TM // (parts * 16)) * 16
        return pl.multiple_of(jnp.minimum(k * size, TM - size), 16), size

    first = i == 0

    @pl.when(first)
    def _():
        start(c_qkv(0), c_qkv(1), c_c(), c_x(0))
        qkv_s[:, :, TM:TM + HALO, :] = jnp.zeros((3, 8, HALO, 128), f32)
        acc_s[...] = jnp.zeros_like(acc_s)
        mod_s[3:5] = jnp.zeros((2, 8, D), f32)

        def perm_body(n, _):
            c_qkv(n).wait()
            pl.when(n == 0)(lambda: start(c_qkv(2), c_mod(0)))
            pl.when(n == 1)(lambda: start(c_mod(1)))
            permute_cols(n)
        jax.lax.fori_loop(0, 3, perm_body, None)

        c_c().wait()

        def mod_body(n, _):
            c_mod(n).wait()
            pl.when(n == 0)(lambda: start(c_wo()))
            pl.when(n == 1)(lambda: start(c_mod(2)))
            mod_part(n)
        jax.lax.fori_loop(0, 2, mod_body, None)
        start(c_x(1), c_mod(3), c_mod(4))
        c_x(0).wait()
        ln1(0, 0, TM)

    @pl.when(i < NT)
    def _():
        if QU:
            ln2(0, TM)
            for n in range(3):
                qkv(n)
        else:
            def body(n, _):
                ln2(*share(n, 3))
                qkv(n)
            jax.lax.fori_loop(0, 3, body, None)

    pl.when(i == NT)(lambda: ln2(0, TM))

    pl.when(i + 2 < NT)(lambda: start(c_x(i + 2)))
    pl.when(i + 1 < NT)(lambda: c_x(i + 1).wait())

    @pl.when(first)
    def _():
        c_wo().wait()
        start(c_mod(5), *c_ffn(0))
        permute_wo()
        def attn_body(t, _):
            for u in range(AU):
                attn(t * AU + u, R0)
        jax.lax.fori_loop(0, TM // (R0 * AU), attn_body, None)

        def body(n, _):
            c_mod(n).wait()
            mod_part(n)
        jax.lax.fori_loop(2, 5, body, None)

    @pl.when(i == 1)
    def _():
        c_mod(5).wait()
        start(*c_ffn(1))
        mod_part(5)

    @pl.when(i > 0)
    def _():
        def body(f, _):
            @pl.when(i == 1)
            def _():
                for c in c_ffn(f):
                    c.wait()
                pl.when(f + 2 < NF)(lambda: start(*c_ffn(f + 2)))
            ffn(f)
            for t in range(per):
                attn(jnp.minimum(f * per + t, nch - 1))
        jax.lax.fori_loop(0, NF, body, None)

    @pl.when(i < NT)
    def _():
        ln1(jnp.minimum(i + 1, NT - 1), 0, TM)
        out_proj()


def _build(S, D, F, TM=256, FC=1792, R=8, NC=256, LR=32, PR=256, AU=2, QU=True, R0=8):
    NT = S // TM
    NF = F // FC
    assert S % TM == 0 and NT >= 2 and F % FC == 0 and NF >= 2 and D == 1024 and TM % R == 0
    bf, f32 = jnp.bfloat16, jnp.float32
    any_spec = pl.BlockSpec(memory_space=pl.ANY)
    call = pl.pallas_call(
        functools.partial(_kernel, TM=TM, NT=NT, R=R, NC=NC, LR=LR, PR=PR, AU=AU, QU=QU, R0=R0),
        grid=(NT + 1,),
        in_specs=[any_spec] * 8,
        out_specs=pl.BlockSpec((TM, D), lambda i: (jnp.maximum(i - 1, 0), 0)),
        out_shape=jax.ShapeDtypeStruct((S, D), bf),
        scratch_shapes=[
            pltpu.VMEM((6, D, D), bf), pltpu.VMEM((3, D, D), bf), pltpu.VMEM((D, D), bf),
            pltpu.VMEM((NF, D, FC), bf), pltpu.VMEM((NF, D, FC), bf), pltpu.VMEM((NF, FC, D), bf),
            pltpu.VMEM((6, 8, D), f32), pltpu.VMEM((TM, D), bf),
            pltpu.VMEM((3, 8, TM + HALO, 128), f32), pltpu.VMEM((TM, D), bf),
            pltpu.VMEM((TM, D), bf), pltpu.VMEM((TM, D), f32),
            pltpu.VMEM((1, D), bf), pltpu.VMEM((NT, TM, D), bf),
            pltpu.SemaphoreType.DMA((10 + 3 * NF,)), pltpu.SemaphoreType.DMA((NT + 1,)),
        ],
        compiler_params=pltpu.CompilerParams(
            dimension_semantics=("arbitrary",), vmem_limit_bytes=100 * 1024 * 1024,
            flags={"XLA_TPU_EVENLY_DISTRIBUTE_CRITICAL_NODES": True}),
    )
    return call


@jax.jit
def pallas_adaLN_cond__sliding_local_dilated__swiglu_ffn__prompt_kernel(
    A_x: jax.Array,
    A_wqkv: jax.Array,
    A_wo: jax.Array,
    B_x: jax.Array,
    B_w_gate: jax.Array,
    B_w_up: jax.Array,
    B_w_down: jax.Array,
    c: jax.Array,
    w_mod: jax.Array,
):
    del B_x
    B, S, D = A_x.shape
    assert B == 1
    out = _build(S, D, B_w_gate.shape[1])(
        c, A_x.reshape(S, D), w_mod, A_wqkv, A_wo, B_w_gate, B_w_up, B_w_down)
    return out.reshape(B, S, D)
```

```python
import functools

import jax
import jax.numpy as jnp
import jax.experimental.pallas as pl
import jax.experimental.pallas.tpu as pltpu

W_WIN, DIL = 8, 2
HALO = 16
LN_EPS = 1e-5


def _layernorm(x):
    m = jnp.mean(x, axis=-1, keepdims=True)
    d = x - m
    v = jnp.mean(d * d, axis=-1, keepdims=True)
    return d * jax.lax.rsqrt(v + LN_EPS)


def _dot(a, b):
    return jnp.dot(a, b, preferred_element_type=jnp.float32)


def _block_transpose(t, axis, unit):
    n = t[0].shape[axis]
    idx = jax.lax.broadcasted_iota(jnp.int32, t[0].shape, axis)
    t = [pltpu.roll(x, unit * g, axis) if g else x for g, x in enumerate(t)]
    for b in range(3):
        bit = (idx & (unit << b)) != 0
        t = [jnp.where(bit, t[(g + (1 << b)) % 8], t[g]) for g in range(8)]
    return [pltpu.roll(t[-s % 8], n - unit * s, axis) if s else t[0] for s in range(8)]


def _kernel(c_hbm, x_hbm, wmod_hbm, wqkv_hbm, wo_hbm, wg_hbm, wu_hbm, wd_hbm,
            o_ref,
            wmod_s, wqkv_s, wo_s, wg_s, wu_s, wd_s,
            mod_s, h_s, qkv_s, att_s, h2_s, acc_s, c_ref, x_s, sems, io_sems,
            *, TM, NT, R, NC, LR, PR, AU, PU, R0):
    i = pl.program_id(0)
    D = x_s.shape[-1]
    NF, _, FC = wg_s.shape
    scale = (D // 32) ** -0.5
    f32, bf16 = jnp.float32, jnp.bfloat16
    nch = TM // R
    per = -(-nch // NF)

    def c_mod(n):
        return pltpu.make_async_copy(
            wmod_hbm.at[:, pl.ds(pl.multiple_of(n * D, D), D)], wmod_s.at[n], sems.at[n])

    def c_qkv(n):
        return pltpu.make_async_copy(
            wqkv_hbm.at[:, pl.ds(pl.multiple_of(n * D, D), D)], wqkv_s.at[n], sems.at[6 + n])

    def c_wo():
        return pltpu.make_async_copy(wo_hbm, wo_s, sems.at[9])

    def c_ffn(f):
        f0 = pl.multiple_of(f * FC, FC)
        return (pltpu.make_async_copy(wg_hbm.at[:, pl.ds(f0, FC)], wg_s.at[f], sems.at[10 + 3 * f]),
                pltpu.make_async_copy(wu_hbm.at[:, pl.ds(f0, FC)], wu_s.at[f], sems.at[11 + 3 * f]),
                pltpu.make_async_copy(wd_hbm.at[pl.ds(f0, FC), :], wd_s.at[f], sems.at[12 + 3 * f]))

    def c_x(t):
        return pltpu.make_async_copy(
            x_hbm.at[pl.ds(pl.multiple_of(t * TM, TM), TM)], x_s.at[t], io_sems.at[t])

    def c_c():
        return pltpu.make_async_copy(c_hbm, c_ref, io_sems.at[NT])

    def start(*cs):
        for c in cs:
            c.start()

    def mod_part(n):
        cv = c_ref[...].astype(f32)
        sc = jnp.broadcast_to((cv * jax.nn.sigmoid(cv)).astype(bf16), (16, D))
        mod_s[n] = _dot(sc, wmod_s[n])[0:8]

    def mod(n):
        return mod_s[n, 0:1, :]

    def permute_cols(n, unroll=False):
        def body(r, _):
            rows = pl.ds(pl.multiple_of(r * PR, PR), PR)
            t = [pltpu.bitcast(wqkv_s[n, rows, g * 128:(g + 1) * 128], jnp.uint32) for g in range(8)]
            t = _block_transpose(t, 1, 4)
            for g in range(8):
                wqkv_s[n, rows, g * 128:(g + 1) * 128] = pltpu.bitcast(t[g], bf16)
        jax.lax.fori_loop(0, D // PR, body, None, unroll=unroll)

    def permute_wo():
        def body(n, _):
            cs = pl.ds(pl.multiple_of(n * 128, 128), 128)
            t = [pltpu.bitcast(wo_s[g * 128:(g + 1) * 128, cs], jnp.uint32) for g in range(8)]
            t = _block_transpose(t, 0, 2)
            for g in range(8):
                wo_s[g * 128:(g + 1) * 128, cs] = pltpu.bitcast(t[g], bf16)
        jax.lax.fori_loop(0, D // 128, body, None)

    def ln1(tile):
        sa, ca1 = mod(0), 1.0 + mod(1)
        for r0 in range(0, TM, LR):
            rows = slice(r0, r0 + LR)
            h_s[rows, :] = (_layernorm(x_s[tile, rows, :].astype(f32)) * ca1 + sa).astype(bf16)

    def qkv(n, first=False):
        if n > 0:
            qkv_s[n, :, 0:HALO, :] = (jnp.zeros((8, HALO, 128), f32) if first
                                      else qkv_s[n, :, TM:TM + HALO, :])
        for c0 in range(0, D, NC):
            y = _dot(h_s[...], wqkv_s[n, :, c0:c0 + NC])
            for jj in range(NC // 128):
                qkv_s[n, c0 // 128 + jj, HALO:HALO + TM, :] = y[:, jj * 128:(jj + 1) * 128]

    def attn(ch, R=R):
        r0 = pl.multiple_of(ch * R, R)

        def rows(n, j, back):
            return qkv_s[n, j, pl.ds(r0 + (HALO - back), R), :]
        l = [None] * W_WIN
        for j in range(8):
            qj = rows(0, j, 0)
            for w in range(W_WIN):
                p = qj * rows(1, j, DIL * w)
                l[w] = p if l[w] is None else l[w] + p
        lane = jax.lax.broadcasted_iota(jnp.int32, (R, 128), 1)
        pos = jax.lax.broadcasted_iota(jnp.int32, (R, 128), 0) + (i * TM + r0)
        b0, b1 = (lane & 1) == 0, (lane & 2) == 0
        for w in range(W_WIN):
            t = l[w]
            t = t + jnp.where(b0, pltpu.roll(t, 127, 1), pltpu.roll(t, 1, 1))
            t = t + jnp.where(b1, pltpu.roll(t, 126, 1), pltpu.roll(t, 2, 1))
            t = t * scale
            l[w] = jnp.where(pos >= DIL * w, t, -1e9) if w else t
        m = functools.reduce(jnp.maximum, l)
        e = [jnp.exp(t - m) for t in l]
        inv = 1.0 / functools.reduce(jnp.add, e)
        e = [t * inv for t in e]
        for j in range(8):
            acc = None
            for w in range(W_WIN):
                p = e[w] * rows(2, j, DIL * w)
                acc = p if acc is None else acc + p
            att_s[pl.ds(r0, R), j * 128:(j + 1) * 128] = acc.astype(bf16)

    def out_proj():
        ga = mod(2)
        for c0 in range(0, D, NC):
            cs = slice(c0, c0 + NC)
            acc_s[:, cs] = x_s[i, :, cs].astype(f32) + ga[:, cs] * _dot(att_s[...], wo_s[:, cs])

    def ln2():
        sb, cb1 = mod(3), 1.0 + mod(4)
        for r0 in range(0, TM, LR):
            rows = slice(r0, r0 + LR)
            h2_s[rows, :] = (_layernorm(acc_s[rows, :]) * cb1 + sb).astype(bf16)

    def ffn(f):
        a = []
        for c0 in range(0, FC, NC):
            cs = slice(c0, min(c0 + NC, FC))
            g = _dot(h2_s[...], wg_s[f, :, cs])
            u = _dot(h2_s[...], wu_s[f, :, cs])
            t = 0.5 * g
            a.append(((t * jnp.tanh(t) + t) * u).astype(bf16))
        a = jnp.concatenate(a, axis=1)
        gb = mod(5)
        for c0 in range(0, D, NC):
            cs = slice(c0, c0 + NC)
            res = acc_s[:, cs] + gb[:, cs] * _dot(a, wd_s[f, :, cs])
            acc_s[:, cs] = res
            o_ref[:, cs] = res.astype(o_ref.dtype)

    @pl.when(i == 0)
    def _():
        start(c_qkv(0), c_qkv(1), c_c(), c_x(0))

        def perm_body(n, _):
            c_qkv(n).wait()
            start(c_mod(n))
            permute_cols(n)
        jax.lax.fori_loop(0, 2, perm_body, None)
        c_c().wait()

        def mod_body(n, _):
            c_mod(n).wait()
            pl.when(n == 0)(lambda: start(c_qkv(2)))
            pl.when(n == 1)(lambda: start(c_wo()))
            mod_part(n)
        jax.lax.fori_loop(0, 2, mod_body, None)
        c_x(0).wait()
        ln1(0)
        qkv(0)
        c_qkv(2).wait()
        start(c_mod(2), c_mod(3), c_x(1))
        permute_cols(2, PU)
        qkv(1, True)
        ffn0 = c_ffn(0)
        start(c_mod(4), *ffn0[:2])
        qkv(2, True)
        c_wo().wait()
        start(c_mod(5), ffn0[2])
        permute_wo()

        def attn_body(t, _):
            for u in range(AU):
                attn(t * AU + u, R0)
        jax.lax.fori_loop(0, TM // (R0 * AU), attn_body, None)

        def mod_body2(n, _):
            c_mod(n).wait()
            mod_part(n)
        jax.lax.fori_loop(2, 5, mod_body2, None)

    @pl.when(i == 1)
    def _():
        c_mod(5).wait()
        start(*c_ffn(1))
        mod_part(5)

    @pl.when(i > 0)
    def _():
        def body(f, _):
            @pl.when(i == 1)
            def _():
                for c in c_ffn(f):
                    c.wait()
                if NF > 2:
                    pl.when(f + 2 < NF)(lambda: start(*c_ffn(f + 2)))
            ffn(f)
            for t in range(per):
                attn(jnp.minimum(f * per + t, nch - 1))
        jax.lax.fori_loop(0, NF, body, None)

    pl.when(i + 1 < NT)(lambda: c_x(i + 1).wait())
    pl.when(i + 2 < NT)(lambda: start(c_x(i + 2)))

    @pl.when(i < NT)
    def _():
        ln1(jnp.minimum(i + 1, NT - 1))
        out_proj()

    @pl.when(i + 1 < NT)
    def _():
        ln2()
        for n in range(3):
            qkv(n)

    pl.when(i + 1 == NT)(ln2)


def _build(S, D, F, TM=256, FC=1792, R=8, NC=256, LR=32, PR=256, AU=2, PU=True, R0=8):
    NT = S // TM
    NF = F // FC
    assert S % TM == 0 and NT >= 2 and F % FC == 0 and NF >= 2 and D == 1024 and TM % R == 0
    bf, f32 = jnp.bfloat16, jnp.float32
    any_spec = pl.BlockSpec(memory_space=pl.ANY)
    call = pl.pallas_call(
        functools.partial(_kernel, TM=TM, NT=NT, R=R, NC=NC, LR=LR, PR=PR, AU=AU, PU=PU, R0=R0),
        grid=(NT + 1,),
        in_specs=[any_spec] * 8,
        out_specs=pl.BlockSpec((TM, D), lambda i: (jnp.maximum(i - 1, 0), 0)),
        out_shape=jax.ShapeDtypeStruct((S, D), bf),
        scratch_shapes=[
            pltpu.VMEM((6, D, D), bf), pltpu.VMEM((3, D, D), bf), pltpu.VMEM((D, D), bf),
            pltpu.VMEM((NF, D, FC), bf), pltpu.VMEM((NF, D, FC), bf), pltpu.VMEM((NF, FC, D), bf),
            pltpu.VMEM((6, 8, D), f32), pltpu.VMEM((TM, D), bf),
            pltpu.VMEM((3, 8, TM + HALO, 128), f32), pltpu.VMEM((TM, D), bf),
            pltpu.VMEM((TM, D), bf), pltpu.VMEM((TM, D), f32),
            pltpu.VMEM((1, D), bf), pltpu.VMEM((NT, TM, D), bf),
            pltpu.SemaphoreType.DMA((10 + 3 * NF,)), pltpu.SemaphoreType.DMA((NT + 1,)),
        ],
        compiler_params=pltpu.CompilerParams(
            dimension_semantics=("arbitrary",), vmem_limit_bytes=100 * 1024 * 1024,
            flags={"XLA_TPU_EVENLY_DISTRIBUTE_CRITICAL_NODES": True}),
    )
    return call


@jax.jit
def pallas_adaLN_cond__sliding_local_dilated__swiglu_ffn__prompt_kernel(
    A_x: jax.Array,
    A_wqkv: jax.Array,
    A_wo: jax.Array,
    B_x: jax.Array,
    B_w_gate: jax.Array,
    B_w_up: jax.Array,
    B_w_down: jax.Array,
    c: jax.Array,
    w_mod: jax.Array,
):
    del B_x
    B, S, D = A_x.shape
    assert B == 1
    out = _build(S, D, B_w_gate.shape[1])(
        c, A_x.reshape(S, D), w_mod, A_wqkv, A_wo, B_w_gate, B_w_up, B_w_down)
    return out.reshape(B, S, D)
```

```python
import functools

import jax
import jax.numpy as jnp
import jax.experimental.pallas as pl
import jax.experimental.pallas.tpu as pltpu

W_WIN, DIL = 8, 2
HALO = 16
LN_EPS = 1e-5


def _layernorm(x):
    m = jnp.mean(x, axis=-1, keepdims=True)
    d = x - m
    v = jnp.mean(d * d, axis=-1, keepdims=True)
    return d * jax.lax.rsqrt(v + LN_EPS)


def _dot(a, b):
    return jnp.dot(a, b, preferred_element_type=jnp.float32)


def _block_transpose(t, axis, unit):
    n = t[0].shape[axis]
    idx = jax.lax.broadcasted_iota(jnp.int32, t[0].shape, axis)
    t = [pltpu.roll(x, unit * g, axis) if g else x for g, x in enumerate(t)]
    for b in range(3):
        bit = (idx & (unit << b)) != 0
        t = [jnp.where(bit, t[(g + (1 << b)) % 8], t[g]) for g in range(8)]
    return [pltpu.roll(t[-s % 8], n - unit * s, axis) if s else t[0] for s in range(8)]


def _kernel(c_hbm, x_hbm, wmod_hbm, wqkv_hbm, wo_hbm, wg_hbm, wu_hbm, wd_hbm,
            o_ref,
            wmod_s, wqkv_s, wo_s, wg_s, wu_s, wd_s,
            mod_s, h_s, qkv_s, att_s, h2_s, acc_s, c_ref, x_s, sems, io_sems,
            *, TM, NT, R, NC, LR, PR, AU):
    i = pl.program_id(0)
    D = x_s.shape[-1]
    NF, _, FC = wg_s.shape
    scale = (D // 32) ** -0.5
    f32, bf16 = jnp.float32, jnp.bfloat16
    nch = TM // R
    per = -(-nch // NF)

    def c_mod(n):
        return pltpu.make_async_copy(
            wmod_hbm.at[:, pl.ds(pl.multiple_of(n * D, D), D)], wmod_s.at[n], sems.at[n])

    def c_qkv(n):
        return pltpu.make_async_copy(
            wqkv_hbm.at[:, pl.ds(pl.multiple_of(n * D, D), D)], wqkv_s.at[n], sems.at[6 + n])

    def c_wo():
        return pltpu.make_async_copy(wo_hbm, wo_s, sems.at[9])

    def c_ffn(f):
        f0 = pl.multiple_of(f * FC, FC)
        return (pltpu.make_async_copy(wg_hbm.at[:, pl.ds(f0, FC)], wg_s.at[f], sems.at[10 + 3 * f]),
                pltpu.make_async_copy(wu_hbm.at[:, pl.ds(f0, FC)], wu_s.at[f], sems.at[11 + 3 * f]),
                pltpu.make_async_copy(wd_hbm.at[pl.ds(f0, FC), :], wd_s.at[f], sems.at[12 + 3 * f]))

    def c_x(t):
        return pltpu.make_async_copy(
            x_hbm.at[pl.ds(pl.multiple_of(t * TM, TM), TM)], x_s.at[t], io_sems.at[t])

    def c_c():
        return pltpu.make_async_copy(c_hbm, c_ref, io_sems.at[NT])

    def start(*cs):
        for c in cs:
            c.start()

    def mod_part(n):
        cv = c_ref[...].astype(f32)
        sc = jnp.broadcast_to((cv * jax.nn.sigmoid(cv)).astype(bf16), (16, D))
        mod_s[n] = _dot(sc, wmod_s[n])[0:8]

    def mod(n):
        return mod_s[n, 0:1, :]

    def permute_cols(n, unroll=False):
        def body(r, _):
            rows = pl.ds(pl.multiple_of(r * PR, PR), PR)
            t = [pltpu.bitcast(wqkv_s[n, rows, g * 128:(g + 1) * 128], jnp.uint32) for g in range(8)]
            t = _block_transpose(t, 1, 4)
            for g in range(8):
                wqkv_s[n, rows, g * 128:(g + 1) * 128] = pltpu.bitcast(t[g], bf16)
        jax.lax.fori_loop(0, D // PR, body, None, unroll=unroll)

    def permute_wo():
        def body(n, _):
            cs = pl.ds(pl.multiple_of(n * 128, 128), 128)
            t = [pltpu.bitcast(wo_s[g * 128:(g + 1) * 128, cs], jnp.uint32) for g in range(8)]
            t = _block_transpose(t, 0, 2)
            for g in range(8):
                wo_s[g * 128:(g + 1) * 128, cs] = pltpu.bitcast(t[g], bf16)
        jax.lax.fori_loop(0, D // 128, body, None)

    def ln1(tile):
        sa, ca1 = mod(0), 1.0 + mod(1)
        for r0 in range(0, TM, LR):
            rows = slice(r0, r0 + LR)
            h_s[rows, :] = (_layernorm(x_s[tile, rows, :].astype(f32)) * ca1 + sa).astype(bf16)

    def qkv(n, first=False):
        if n > 0:
            qkv_s[n, :, 0:HALO, :] = (jnp.zeros((8, HALO, 128), f32) if first
                                      else qkv_s[n, :, TM:TM + HALO, :])
        for c0 in range(0, D, NC):
            y = _dot(h_s[...], wqkv_s[n, :, c0:c0 + NC])
            for jj in range(NC // 128):
                qkv_s[n, c0 // 128 + jj, HALO:HALO + TM, :] = y[:, jj * 128:(jj + 1) * 128]

    def attn(ch):
        r0 = pl.multiple_of(ch * R, R)

        def rows(n, j, back):
            return qkv_s[n, j, pl.ds(r0 + (HALO - back), R), :]
        l = [None] * W_WIN
        for j in range(8):
            qj = rows(0, j, 0)
            for w in range(W_WIN):
                p = qj * rows(1, j, DIL * w)
                l[w] = p if l[w] is None else l[w] + p
        lane = jax.lax.broadcasted_iota(jnp.int32, (R, 128), 1)
        pos = jax.lax.broadcasted_iota(jnp.int32, (R, 128), 0) + (i * TM + r0)
        b0, b1 = (lane & 1) == 0, (lane & 2) == 0
        for w in range(W_WIN):
            t = l[w]
            t = t + jnp.where(b0, pltpu.roll(t, 127, 1), pltpu.roll(t, 1, 1))
            t = t + jnp.where(b1, pltpu.roll(t, 126, 1), pltpu.roll(t, 2, 1))
            t = t * scale
            l[w] = jnp.where(pos >= DIL * w, t, -1e9) if w else t
        m = functools.reduce(jnp.maximum, l)
        e = [jnp.exp(t - m) for t in l]
        inv = 1.0 / functools.reduce(jnp.add, e)
        e = [t * inv for t in e]
        for j in range(8):
            acc = None
            for w in range(W_WIN):
                p = e[w] * rows(2, j, DIL * w)
                acc = p if acc is None else acc + p
            att_s[pl.ds(r0, R), j * 128:(j + 1) * 128] = acc.astype(bf16)

    def out_proj():
        ga = mod(2)
        for c0 in range(0, D, NC):
            cs = slice(c0, c0 + NC)
            acc_s[:, cs] = x_s[i, :, cs].astype(f32) + ga[:, cs] * _dot(att_s[...], wo_s[:, cs])

    def ln2():
        sb, cb1 = mod(3), 1.0 + mod(4)
        for r0 in range(0, TM, LR):
            rows = slice(r0, r0 + LR)
            h2_s[rows, :] = (_layernorm(acc_s[rows, :]) * cb1 + sb).astype(bf16)

    def ffn(f):
        a = []
        for c0 in range(0, FC, NC):
            cs = slice(c0, min(c0 + NC, FC))
            g = _dot(h2_s[...], wg_s[f, :, cs])
            u = _dot(h2_s[...], wu_s[f, :, cs])
            t = 0.5 * g
            a.append(((t * jnp.tanh(t) + t) * u).astype(bf16))
        a = jnp.concatenate(a, axis=1)
        gb = mod(5)
        for c0 in range(0, D, NC):
            cs = slice(c0, c0 + NC)
            res = acc_s[:, cs] + gb[:, cs] * _dot(a, wd_s[f, :, cs])
            acc_s[:, cs] = res
            o_ref[:, cs] = res.astype(o_ref.dtype)

    @pl.when(i == 0)
    def _():
        start(c_qkv(0), c_qkv(1), c_c(), c_x(0))

        def perm_body(n, _):
            c_qkv(n).wait()
            start(c_mod(n))
            permute_cols(n)
        jax.lax.fori_loop(0, 2, perm_body, None)
        c_c().wait()

        def mod_body(n, _):
            c_mod(n).wait()
            pl.when(n == 0)(lambda: start(c_qkv(2)))
            pl.when(n == 1)(lambda: start(c_wo()))
            mod_part(n)
        jax.lax.fori_loop(0, 2, mod_body, None)
        c_x(0).wait()
        ln1(0)
        qkv(0)
        c_qkv(2).wait()
        start(c_mod(2), c_mod(3), c_x(1))
        permute_cols(2, unroll=True)
        qkv(1, True)
        start(c_mod(4), c_mod(5))
        qkv(2, True)
        c_wo().wait()
        start(*c_ffn(0))
        permute_wo()

        def attn_body(t, _):
            for u in range(AU):
                attn(t * AU + u)
        jax.lax.fori_loop(0, nch // AU, attn_body, None)

        def mod_body2(n, _):
            c_mod(n).wait()
            mod_part(n)
        jax.lax.fori_loop(2, 6, mod_body2, None)
        start(*c_ffn(1))

    @pl.when(i > 0)
    def _():
        def body(f, _):
            @pl.when(i == 1)
            def _():
                for c in c_ffn(f):
                    c.wait()
                if NF > 2:
                    pl.when(f + 2 < NF)(lambda: start(*c_ffn(f + 2)))
            ffn(f)
            for t in range(per):
                attn(jnp.minimum(f * per + t, nch - 1))
        jax.lax.fori_loop(0, NF, body, None)

    pl.when(i + 1 < NT)(lambda: c_x(i + 1).wait())
    pl.when(i + 2 < NT)(lambda: start(c_x(i + 2)))

    @pl.when(i < NT)
    def _():
        ln1(jnp.minimum(i + 1, NT - 1))
        out_proj()

    @pl.when(i + 1 < NT)
    def _():
        ln2()
        for n in range(3):
            qkv(n)

    pl.when(i + 1 == NT)(ln2)


def _build(S, D, F, TM=256, FC=1792, R=8, NC=128, LR=32, PR=256, AU=2):
    NT = S // TM
    NF = F // FC
    assert S % TM == 0 and NT >= 2 and F % FC == 0 and NF >= 2 and D == 1024 and TM % R == 0
    bf, f32 = jnp.bfloat16, jnp.float32
    any_spec = pl.BlockSpec(memory_space=pl.ANY)
    call = pl.pallas_call(
        functools.partial(_kernel, TM=TM, NT=NT, R=R, NC=NC, LR=LR, PR=PR, AU=AU),
        grid=(NT + 1,),
        in_specs=[any_spec] * 8,
        out_specs=pl.BlockSpec((TM, D), lambda i: (jnp.maximum(i - 1, 0), 0)),
        out_shape=jax.ShapeDtypeStruct((S, D), bf),
        scratch_shapes=[
            pltpu.VMEM((6, D, D), bf), pltpu.VMEM((3, D, D), bf), pltpu.VMEM((D, D), bf),
            pltpu.VMEM((NF, D, FC), bf), pltpu.VMEM((NF, D, FC), bf), pltpu.VMEM((NF, FC, D), bf),
            pltpu.VMEM((6, 8, D), f32), pltpu.VMEM((TM, D), bf),
            pltpu.VMEM((3, 8, TM + HALO, 128), f32), pltpu.VMEM((TM, D), bf),
            pltpu.VMEM((TM, D), bf), pltpu.VMEM((TM, D), f32),
            pltpu.VMEM((1, D), bf), pltpu.VMEM((NT, TM, D), bf),
            pltpu.SemaphoreType.DMA((10 + 3 * NF,)), pltpu.SemaphoreType.DMA((NT + 1,)),
        ],
        compiler_params=pltpu.CompilerParams(
            dimension_semantics=("arbitrary",), vmem_limit_bytes=100 * 1024 * 1024,
            flags={"XLA_TPU_EVENLY_DISTRIBUTE_CRITICAL_NODES": True}),
    )
    return call


@jax.jit
def pallas_adaLN_cond__sliding_local_dilated__swiglu_ffn__prompt_kernel(
    A_x: jax.Array,
    A_wqkv: jax.Array,
    A_wo: jax.Array,
    B_x: jax.Array,
    B_w_gate: jax.Array,
    B_w_up: jax.Array,
    B_w_down: jax.Array,
    c: jax.Array,
    w_mod: jax.Array,
):
    del B_x
    B, S, D = A_x.shape
    assert B == 1
    out = _build(S, D, B_w_gate.shape[1])(
        c, A_x.reshape(S, D), w_mod, A_wqkv, A_wo, B_w_gate, B_w_up, B_w_down)
    return out.reshape(B, S, D)
```
